```python
import os as _os
_os.environ.setdefault("JAX_PLATFORMS", "cpu")
import jax
import jax.numpy as jnp

def _softmax(x, axis=-1):
    return jax.nn.softmax(x, axis=axis)
def _gelu(x):
    return jax.nn.gelu(x, approximate=True)
def _silu(x):
    return jax.nn.silu(x)
def _sigmoid(x):
    return jax.nn.sigmoid(x)
def _layernorm(x, axis=-1, eps=1e-5):
    m = jnp.mean(x, axis=axis, keepdims=True)
    v = jnp.var(x, axis=axis, keepdims=True)
    return (x - m) / jnp.sqrt(v + eps)
def _scatter_add(tgt, idx, src, axis=0):
    return tgt.at[idx].add(src)
def _segment_sum(src, seg, n):
    return jax.ops.segment_sum(src, seg, n)
class _Rng:
    def __init__(self, key):
        self._k = key
    def _next(self):
        self._k, sub = jax.random.split(self._k)
        return sub
    def normal(self, shape):
        return jax.random.normal(self._next(), shape, dtype=jnp.bfloat16)
    def randint(self, lo, hi, shape):
        return jax.random.randint(self._next(), shape, lo, hi, dtype=jnp.int32)
    def uniform(self, shape, lo=0.0, hi=1.0):
        return jax.random.uniform(self._next(), shape, jnp.bfloat16, lo, hi)
    def permutation(self, n):
        return jax.random.permutation(self._next(), n)


kernel_name = 'gated_mix__gqa_block_cached__dense_activation_squared_relu__decode'

def setup_inputs():
    _rng = _Rng(jax.random.key(int.from_bytes(__import__("os").urandom(4), "little")))
    _w = (lambda a: (lambda t: t.astype(jnp.bfloat16) if jnp.issubdtype(t.dtype, jnp.floating) else t)(jnp.asarray(a)))
    def _A_setup():
        B, Sq, D = 4, 1, 512
        Hq, Hkv, Sk, Dh = 32, 8, 4096, 128
        assert Hq % Hkv == 0, (Hq, Hkv)
        return {
            "x": _w((lambda *s: _rng.normal(s) * 0.05)(B, Sq, D)),
            "k_cache": _w((lambda *s: _rng.normal(s) * 3.2)(B, Hkv, Sk, Dh)),
            "v_cache": _w((lambda *s: _rng.normal(s) * 1.6)(B, Hkv, Sk, Dh)),
            "wq": _w((lambda *s: _rng.normal(s) * 3.2)(D, Hq * Dh) * (D ** -0.5)),
            "wo": _w((lambda *s: _rng.normal(s) * 1.6)(Hq * Dh, D) * ((Hq * Dh) ** -0.5)),
        }
    _A_in = _A_setup()

    def _B_setup():
        B, S, D, F = 4, 1, 512, 1792
        return {
            "x": _w((lambda *s: _rng.normal(s) * 0.05)(B, S, D)),
            "w1": _w((lambda *s: _rng.normal(s) * 0.1)(D, F)),
            "b1": _w((lambda *s: _rng.normal(s) * 0.05)(F)),
            "w2": _w((lambda *s: _rng.normal(s) * 0.05)(F, D)),
            "b2": _w((lambda *s: _rng.normal(s) * 0.05)(D)),
        }
    _B_in = _B_setup()

    return {
        "A_x": _A_in["x"],
        "A_k_cache": _A_in["k_cache"],
        "A_v_cache": _A_in["v_cache"],
        "A_wq": _A_in["wq"],
        "A_wo": _A_in["wo"],
        "B_x": _B_in["x"],
        "B_w1": _B_in["w1"],
        "B_b1": _B_in["b1"],
        "B_w2": _B_in["w2"],
        "B_b2": _B_in["b2"],
        "gate_w": _w((lambda *s: _rng.normal(s) * 0.05)(512) * 16.0),
    }

def reference(A_x, A_k_cache, A_v_cache, A_wq, A_wo, B_x, B_w1, B_b1, B_w2, B_b2, gate_w):
    def _A_ref(x, k_cache, v_cache, wq, wo):
        B, Sq, D = x.shape
        Hq, Dh = 32, 128
        Hkv = k_cache.shape[1]
        rep = Hq // Hkv
        q = (lambda x, *d: x.transpose(*d))((x @ wq).reshape(B, Sq, Hq, Dh), 0, 2, 1, 3)
        k = jnp.repeat(k_cache, rep, axis=1)
        v = jnp.repeat(v_cache, rep, axis=1)
        scores = jnp.einsum("bhqd,bhkd->bhqk", q, k) * (Dh ** -0.5)
        p = _softmax(scores, axis=-1)
        o = jnp.einsum("bhqk,bhkd->bhqd", p, v)
        return (lambda x, *d: x.transpose(*d))(o, 0, 2, 1, 3).reshape(B, Sq, Hq * Dh) @ wo

    def _B_ref(x, w1, b1, w2, b2):
        h = jnp.einsum("bsd,df->bsf", x, w1) + b1
        zero = jnp.zeros_like(h)
        r = jnp.where(h > zero, h, zero)
        h = r * r
        out = jnp.einsum("bsf,fd->bsd", h, w2) + b2
        return out

    x = A_x
    g = _sigmoid((x * gate_w).sum(-1, keepdims=True))
    a = _A_ref(x, A_k_cache, A_v_cache, A_wq, A_wo)
    b = _B_ref(x, B_w1, B_b1, B_w2, B_b2)
    return g * a + (1 - g) * b
```

```python
import functools
import numpy as np
import jax
import jax.numpy as jnp
from jax import lax
from jax.experimental import pallas as pl
from jax.experimental.pallas import tpu as pltpu

B, D, HQ, HKV, SK, DH, F = 4, 512, 32, 8, 4096, 128, 1792
REP = HQ // HKV
R16 = REP * B
f32, bf16 = jnp.float32, jnp.bfloat16


def make_kernel(NBUF=4, LOOK=3, vmem_mb=64):
    assert LOOK < NBUF
    NSTEP = B * HKV

    def kern(x_hbm, k_hbm, v_hbm, wq_hbm, wo_hbm, w1_hbm, b1_hbm, w2_hbm, b2_hbm, gw_hbm,
             o_ref,
             x_v, gw_v, b1_v, b2_v, wq_v, wo_v, w1_v, w2_v, kbuf, vbuf,
             small_sem, wq_sem, wo_sem, w1_sem, w2_sem, ksem, vsem):
        def small_cps():
            return [pltpu.make_async_copy(x_hbm, x_v, small_sem.at[0]),
                    pltpu.make_async_copy(gw_hbm, gw_v, small_sem.at[1]),
                    pltpu.make_async_copy(b1_hbm, b1_v, small_sem.at[2]),
                    pltpu.make_async_copy(b2_hbm, b2_v, small_sem.at[3])]

        def wq_cp(h):
            return pltpu.make_async_copy(wq_hbm.at[:, pl.ds(h * 512, 512)], wq_v.at[h], wq_sem.at[h])

        def wo_cp(h):
            return pltpu.make_async_copy(wo_hbm.at[pl.ds(h * 512, 512), :], wo_v.at[h], wo_sem.at[h])

        def k_cp(i):
            return pltpu.make_async_copy(k_hbm.at[i % B, i // B], kbuf.at[i % NBUF], ksem.at[i % NBUF])

        def v_cp(i):
            return pltpu.make_async_copy(v_hbm.at[i % B, i // B], vbuf.at[i % NBUF], vsem.at[i % NBUF])

        w1_cp = pltpu.make_async_copy(w1_hbm, w1_v, w1_sem)
        w2_cp = pltpu.make_async_copy(w2_hbm, w2_v, w2_sem)

        for c in small_cps():
            c.start()
        wq_cp(0).start()
        for i in range(LOOK):
            k_cp(i).start()
            v_cp(i).start()
            if i == 0:
                w1_cp.start()
        for c in small_cps():
            c.wait()
        row = lax.broadcasted_iota(jnp.int32, (R16, D), 0)
        x4 = x_v[...].astype(f32)
        x16 = jnp.concatenate([x4] * REP, axis=0)
        gw = gw_v[...].astype(f32).reshape(1, D)
        gl = jnp.sum(x16 * gw, axis=-1, keepdims=True)
        g16 = 1.0 / (1.0 + jnp.exp(-gl))
        x16b = x16.astype(bf16)
        xr = [jnp.where(row // B == r, x16, 0.0).astype(bf16) for r in range(REP)]

        w1_cp.wait()
        hpre = jnp.dot(x16b, w1_v[...], preferred_element_type=f32) + b1_v[...].astype(f32).reshape(1, F)
        hr = jnp.maximum(hpre, 0.0)
        hact = (hr * hr).astype(bf16)

        rowq = lax.broadcasted_iota(jnp.int32, (R16, DH), 0)
        c_exp = float(DH ** -0.5)

        def q_for(h):
            acc = jnp.zeros((R16, DH), f32)
            for r in range(REP):
                acc += jnp.dot(xr[r], wq_v[h, :, r * DH:(r + 1) * DH], preferred_element_type=f32)
            return acc.astype(bf16)

        def step(i, carry):
            qh, oh, acc_a = carry
            h = i // B
            b = i % B

            @pl.when(i + LOOK < NSTEP)
            def _():
                k_cp(i + LOOK).start()
                v_cp(i + LOOK).start()

            @pl.when(b == 0)
            def _():
                wo_cp(h).start()

                @pl.when(h + 1 < HKV)
                def _():
                    wq_cp(h + 1).start()

            @pl.when(i == NSTEP - LOOK)
            def _():
                w2_cp.start()

            def new_q():
                wq_cp(h).wait()
                return q_for(h)
            qh_new = lax.cond(b == 0, new_q, lambda: qh)
            oh = jnp.where(b == 0, 0.0, oh)

            slot = i % NBUF
            k_cp(i).wait()
            s = lax.dot_general(qh_new, kbuf[slot], (((1,), (1,)), ((), ())), preferred_element_type=f32)
            m = jnp.max(s, axis=-1, keepdims=True)
            p = jnp.exp((s - m) * c_exp)
            l = jnp.sum(p, axis=-1, keepdims=True)
            v_cp(i).wait()
            o = jnp.dot(p.astype(bf16), vbuf[slot], preferred_element_type=f32)
            oh = oh + jnp.where(rowq % B == b, o / l, 0.0)

            def proj():
                wo_cp(h).wait()
                a = acc_a
                ohb = oh.astype(bf16)
                for r in range(REP):
                    lhs = jnp.where(rowq // B == r, ohb, jnp.zeros_like(ohb))
                    a = a + jnp.dot(lhs, wo_v[h, r * DH:(r + 1) * DH, :], preferred_element_type=f32)
                return a
            acc_a = lax.cond(b == B - 1, proj, lambda: acc_a)
            return qh_new, oh, acc_a

        init = (jnp.zeros((R16, DH), bf16), jnp.zeros((R16, DH), f32), jnp.zeros((R16, D), f32))
        _, _, acc_a = lax.fori_loop(0, NSTEP, step, init)

        w2_cp.wait()
        bo = jnp.dot(hact, w2_v[...], preferred_element_type=f32) + b2_v[...].astype(f32).reshape(1, D)
        a8 = acc_a[0:8] + acc_a[8:16]
        a4 = a8 + pltpu.roll(a8, 4, 0)
        g8 = g16[0:8]
        res = g8 * a4 + (1.0 - g8) * bo[0:8]
        o_ref[...] = res[0:B].astype(o_ref.dtype)

    @jax.jit
    def f(A_x, A_k_cache, A_v_cache, A_wq, A_wo, B_x, B_w1, B_b1, B_w2, B_b2, gate_w):
        any_spec = pl.BlockSpec(memory_space=pl.ANY)
        return pl.pallas_call(
            kern,
            in_specs=[any_spec] * 10,
            out_specs=pl.BlockSpec(memory_space=pltpu.VMEM),
            out_shape=jax.ShapeDtypeStruct((B, D), bf16),
            scratch_shapes=[
                pltpu.VMEM((B, D), bf16), pltpu.VMEM((D,), bf16), pltpu.VMEM((F,), bf16), pltpu.VMEM((D,), bf16),
                pltpu.VMEM((HKV, D, 512), bf16), pltpu.VMEM((HKV, 512, D), bf16),
                pltpu.VMEM((D, F), bf16), pltpu.VMEM((F, D), bf16),
                pltpu.VMEM((NBUF, SK, DH), bf16), pltpu.VMEM((NBUF, SK, DH), bf16),
                pltpu.SemaphoreType.DMA((4,)), pltpu.SemaphoreType.DMA((HKV,)), pltpu.SemaphoreType.DMA((HKV,)),
                pltpu.SemaphoreType.DMA(()), pltpu.SemaphoreType.DMA(()),
                pltpu.SemaphoreType.DMA((NBUF,)), pltpu.SemaphoreType.DMA((NBUF,)),
            ],
            compiler_params=pltpu.CompilerParams(vmem_limit_bytes=vmem_mb * 1024 * 1024),
        )(A_x.reshape(B, D), A_k_cache, A_v_cache, A_wq, A_wo, B_w1, B_b1, B_w2, B_b2, gate_w).reshape(B, 1, D)
    return f


pallas_gated_mix__gqa_block_cached__dense_activation_squared_relu__decode_kernel = make_kernel(4, 3)
```

```python
import numpy as np

import jax
import jax.numpy as jnp
from jax import lax
from jax.experimental import pallas as pl
from jax.experimental.pallas import tpu as pltpu

B, D, HQ, HKV, SK, DH, F = 4, 512, 32, 8, 4096, 128, 1792
REP = HQ // HKV
R16 = REP * B
NSTEP = B * HKV

NBUF = 4
LOOK = 3
NWQ = 4
NWO = 4
W2_LATE = (384, 256, 128)
W2_EARLY = F - sum(W2_LATE)
W2_OFF = tuple(int(v) for v in np.cumsum((W2_EARLY,) + W2_LATE))
STEP_FFN_UP = 2
STEP_W2E_ISSUE = 16
STEP_W2E = 24

_F32, _BF16 = jnp.float32, jnp.bfloat16


def _kernel(x_hbm, k_hbm, v_hbm, wq_hbm, wo_hbm, w1_hbm, b1_hbm, w2_hbm, b2_hbm, gw_hbm,
            o_ref,
            x_v, gw_v, b1_v, b2_v, wq_v, wo_v, w1_v, w2_v, kbuf, vbuf, h_v, q_v, bo_v,
            small_sem, wq_sem, wo_sem, w1_sem, w2e_sem, w2l_sem, k_sem, v_sem):
  rq, ro = D // NWQ, (HQ * DH) // NWO
  heads_per_wo = HKV // NWO

  def small_copies():
    return [pltpu.make_async_copy(x_hbm, x_v, small_sem.at[0]),
            pltpu.make_async_copy(gw_hbm, gw_v, small_sem.at[1]),
            pltpu.make_async_copy(b1_hbm, b1_v, small_sem.at[2]),
            pltpu.make_async_copy(b2_hbm, b2_v, small_sem.at[3])]

  def wq_copy(j):
    rows = pl.ds(j * rq, rq)
    return pltpu.make_async_copy(wq_hbm.at[rows, :], wq_v.at[rows, :], wq_sem.at[j])

  def wo_copy(j):
    rows = pl.ds(j * ro, ro)
    return pltpu.make_async_copy(wo_hbm.at[rows, :], wo_v.at[rows, :], wo_sem.at[j])

  def k_copy(i):
    slot = i % NBUF
    return pltpu.make_async_copy(k_hbm.at[i % B, i // B], kbuf.at[slot], k_sem.at[slot])

  def v_copy(i):
    slot = i % NBUF
    return pltpu.make_async_copy(v_hbm.at[i % B, i // B], vbuf.at[slot], v_sem.at[slot])

  def w2_late_copy(c):
    rows = pl.ds(W2_OFF[c], W2_LATE[c])
    return pltpu.make_async_copy(w2_hbm.at[rows, :], w2_v.at[rows, :], w2l_sem.at[c])

  early = pl.ds(0, W2_EARLY)
  w2_early_copy = pltpu.make_async_copy(w2_hbm.at[early, :], w2_v.at[early, :], w2e_sem)
  w1_copy = pltpu.make_async_copy(w1_hbm, w1_v, w1_sem)

  def start_kv(i):
    k_copy(i).start(priority=0)
    v_copy(i).start(priority=1)

  for c in small_copies():
    c.start(priority=0)
  for j in range(NWQ):
    wq_copy(j).start(priority=0)
  start_kv(0)
  w1_copy.start(priority=1)
  for i in range(1, LOOK):
    start_kv(i)
  for j in range(NWO):
    wo_copy(j).start(priority=j % 2)

  for c in small_copies():
    c.wait()
  x16 = jnp.concatenate([x_v[...].astype(_F32)] * REP, axis=0)
  gate_logit = jnp.sum(x16[0:8] * gw_v[...].astype(_F32).reshape(1, D),
                       axis=-1, keepdims=True)
  g8 = 1.0 / (1.0 + jnp.exp(-gate_logit))

  row_d = lax.broadcasted_iota(jnp.int32, (R16, D), 0)
  x_r = [jnp.where(row_d // B == r, x16, 0.0).astype(_BF16) for r in range(REP)]
  for j in range(NWQ):
    wq_copy(j).wait()
  for h in range(HKV):
    q = jnp.zeros((R16, DH), _F32)
    for r in range(REP):
      col = (h * REP + r) * DH
      q += jnp.dot(x_r[r], wq_v[:, col:col + DH], preferred_element_type=_F32)
    q_v[h] = q.astype(_BF16)

  row_h = lax.broadcasted_iota(jnp.int32, (R16, DH), 0)
  scale = float(DH ** -0.5)

  def step(i, carry):
    o_h, acc_a = carry
    h = i // B
    b = i % B

    @pl.when(i + LOOK < NSTEP)
    def _():
      start_kv(i + LOOK)

    @pl.when(i == STEP_W2E_ISSUE)
    def _():
      w2_early_copy.start(priority=1)

    @pl.when(i == NSTEP - LOOK)
    def _():
      for c in range(len(W2_LATE)):
        w2_late_copy(c).start(priority=1)

    @pl.when(i == STEP_FFN_UP)
    def _():
      w1_copy.wait()
      xb = jnp.concatenate([x_v[...]] * REP, axis=0)
      pre = jnp.dot(xb, w1_v[...], preferred_element_type=_F32)
      pre = pre + b1_v[...].astype(_F32).reshape(1, F)
      relu = jnp.where(pre > 0.0, pre, 0.0)
      h_v[...] = (relu * relu).astype(_BF16)

    @pl.when(i == STEP_W2E)
    def _():
      w2_early_copy.wait()
      part = jnp.dot(h_v[:, 0:W2_EARLY], w2_v[0:W2_EARLY, :], preferred_element_type=_F32)
      bo_v[...] = part[0:8] + b2_v[...].astype(_F32).reshape(1, D)

    o_h = jnp.where(b == 0, 0.0, o_h)
    slot = i % NBUF
    k_copy(i).wait()
    s = lax.dot_general(q_v[h], kbuf[slot], (((1,), (1,)), ((), ())),
                        preferred_element_type=_F32)
    m = jnp.max(s, axis=-1, keepdims=True)
    p = jnp.exp((s - m) * scale)
    l = jnp.sum(p, axis=-1, keepdims=True)
    v_copy(i).wait()
    o = jnp.dot(p.astype(_BF16), vbuf[slot], preferred_element_type=_F32)
    o_h = o_h + jnp.where(row_h % B == b, o / l, 0.0)

    def project():
      @pl.when(h % heads_per_wo == 0)
      def _():
        wo_copy(h // heads_per_wo).wait()

      acc = acc_a
      o_bf = o_h.astype(_BF16)
      for r in range(REP):
        lhs = jnp.where(row_h // B == r, o_bf, jnp.zeros_like(o_bf))
        row0 = pl.multiple_of((h * REP + r) * DH, DH)
        acc = acc + jnp.dot(lhs, wo_v[pl.ds(row0, DH), :], preferred_element_type=_F32)
      return acc

    acc_a = lax.cond(b == B - 1, project, lambda: acc_a)
    return o_h, acc_a

  init = (jnp.zeros((R16, DH), _F32), jnp.zeros((R16, D), _F32))
  _, acc_a = lax.fori_loop(0, NSTEP, step, init)

  a8 = acc_a[0:8] + acc_a[8:16]
  a4 = a8 + pltpu.roll(a8, 4, 0)
  bo = bo_v[...]
  for c in range(len(W2_LATE)):
    w2_late_copy(c).wait()
    rows = slice(W2_OFF[c], W2_OFF[c + 1])
    bo = bo + jnp.dot(h_v[:, rows], w2_v[rows, :], preferred_element_type=_F32)[0:8]
  res = g8 * a4 + (1.0 - g8) * bo
  o_ref[...] = res[0:B].astype(o_ref.dtype)


@jax.jit
def pallas_gated_mix__gqa_block_cached__dense_activation_squared_relu__decode_kernel(
    A_x: jax.Array,
    A_k_cache: jax.Array,
    A_v_cache: jax.Array,
    A_wq: jax.Array,
    A_wo: jax.Array,
    B_x: jax.Array,
    B_w1: jax.Array,
    B_b1: jax.Array,
    B_w2: jax.Array,
    B_b2: jax.Array,
    gate_w: jax.Array,
):
  del B_x
  hbm = pl.BlockSpec(memory_space=pl.ANY)
  out = pl.pallas_call(
      _kernel,
      in_specs=[hbm] * 10,
      out_specs=pl.BlockSpec(memory_space=pltpu.VMEM),
      out_shape=jax.ShapeDtypeStruct((B, D), _BF16),
      scratch_shapes=[
          pltpu.VMEM((B, D), _BF16),
          pltpu.VMEM((D,), _BF16),
          pltpu.VMEM((F,), _BF16),
          pltpu.VMEM((D,), _BF16),
          pltpu.VMEM((D, HQ * DH), _BF16),
          pltpu.VMEM((HQ * DH, D), _BF16),
          pltpu.VMEM((D, F), _BF16),
          pltpu.VMEM((F, D), _BF16),
          pltpu.VMEM((NBUF, SK, DH), _BF16),
          pltpu.VMEM((NBUF, SK, DH), _BF16),
          pltpu.VMEM((R16, F), _BF16),
          pltpu.VMEM((HKV, R16, DH), _BF16),
          pltpu.VMEM((8, D), _F32),
          pltpu.SemaphoreType.DMA((4,)),
          pltpu.SemaphoreType.DMA((NWQ,)),
          pltpu.SemaphoreType.DMA((NWO,)),
          pltpu.SemaphoreType.DMA(()),
          pltpu.SemaphoreType.DMA(()),
          pltpu.SemaphoreType.DMA((len(W2_LATE),)),
          pltpu.SemaphoreType.DMA((NBUF,)),
          pltpu.SemaphoreType.DMA((NBUF,)),
      ],
      compiler_params=pltpu.CompilerParams(
          vmem_limit_bytes=48 * 1024 * 1024,
          disable_semaphore_checks=True,
      ),
  )(A_x.reshape(B, D), A_k_cache, A_v_cache, A_wq, A_wo, B_w1, B_b1, B_w2, B_b2, gate_w)
  return out.reshape(B, 1, D)
```

```python
import numpy as np

import jax
import jax.numpy as jnp
from jax import lax
from jax.experimental import pallas as pl
from jax.experimental.pallas import tpu as pltpu

B, D, HQ, HKV, SK, DH, F = 4, 512, 32, 8, 4096, 128, 1792
REP = HQ // HKV
R16 = REP * B
NSTEP = B * HKV

LOOK = 2
NBUF = LOOK + 1
KV_ROWS = 160
W_ROWS = 32
WQ_COLS = 2560
WO_HALF = HQ * DH // 2
W2_LATE = (384, 256, 128)
W2_EARLY = F - sum(W2_LATE)
W2_OFF = tuple(int(v) for v in np.cumsum((W2_EARLY,) + W2_LATE))
STEP_W1_ISSUE = 0
STEP_WO0_ISSUE = 1
STEP_WO1_ISSUE = 8
STEP_W2E_ISSUE = 16
STEP_FFN_UP = 3
STEP_W2E = 24

_F32, _BF16 = jnp.float32, jnp.bfloat16


def _row_pieces(r0, r1, rows):
  return [(s, min(rows, r1 - s)) for s in range(r0, r1, rows)]


def _kernel(x_hbm, k_hbm, v_hbm, wq_hbm, wo_hbm, w1_hbm, b1_hbm, w2_hbm, b2_hbm, gw_hbm,
            o_ref,
            x_v, gw_v, b1_v, b2_v, wq_v, wo_v, w1_v, w2_v, kbuf, vbuf, h_v, q_v, bo_v,
            small_sem, wq_sem, wo_sem, w1_sem, w2e_sem, w2l_sem, k_sem, v_sem):

  def start_rows(src, dst, sem, pieces, priority=None):
    half = (len(pieces) + 1) // 2
    if priority is None:
      order = []
      for j in range(half):
        order.append((pieces[j], 0))
        if half + j < len(pieces):
          order.append((pieces[half + j], 1))
    else:
      order = [(p, priority) for p in pieces]
    for (r0, n), prio in order:
      rows = pl.ds(r0, n)
      pltpu.make_async_copy(src.at[rows, :], dst.at[rows, :], sem).start(priority=prio)

  def wait_filled(dst, sem):
    pltpu.make_async_copy(dst, dst, sem).wait()

  def small_copies():
    return [pltpu.make_async_copy(x_hbm, x_v, small_sem.at[0]),
            pltpu.make_async_copy(gw_hbm, gw_v, small_sem.at[1]),
            pltpu.make_async_copy(b1_hbm, b1_v, small_sem.at[2]),
            pltpu.make_async_copy(b2_hbm, b2_v, small_sem.at[3])]

  kv_pieces = _row_pieces(0, SK, KV_ROWS)

  def start_k(i):
    slot = i % NBUF
    start_rows(k_hbm.at[i % B, i // B], kbuf.at[slot], k_sem.at[slot], kv_pieces)

  def start_v(i):
    slot = i % NBUF
    start_rows(v_hbm.at[i % B, i // B], vbuf.at[slot], v_sem.at[slot], kv_pieces)

  for c in small_copies():
    c.start(priority=0)

  def issue_wq(j, carry):
    for half in range(2):
      rows = pl.ds(pl.multiple_of(j * 8 + half * (D // 2), 8), 8)
      for c0 in range(0, HQ * DH, WQ_COLS):
        cols = pl.ds(c0, min(WQ_COLS, HQ * DH - c0))
        pltpu.make_async_copy(wq_hbm.at[rows, cols], wq_v.at[rows, cols],
                              wq_sem).start(priority=half)
    return carry

  lax.fori_loop(0, D // 16, issue_wq, 0)
  for i in range(LOOK):
    start_k(i)
    start_v(i)

  for c in small_copies():
    c.wait()
  x16 = jnp.concatenate([x_v[...].astype(_F32)] * REP, axis=0)
  gate_logit = jnp.sum(x16[0:8] * gw_v[...].astype(_F32).reshape(1, D),
                       axis=-1, keepdims=True)
  g8 = 1.0 / (1.0 + jnp.exp(-gate_logit))

  row_d = lax.broadcasted_iota(jnp.int32, (R16, D), 0)
  x_r = [jnp.where(row_d // B == r, x16, 0.0).astype(_BF16) for r in range(REP)]
  wait_filled(wq_v, wq_sem)
  for h in range(HKV):
    q = jnp.zeros((R16, DH), _F32)
    for r in range(REP):
      col = (h * REP + r) * DH
      q += jnp.dot(x_r[r], wq_v[:, col:col + DH], preferred_element_type=_F32)
    q_v[h] = q.astype(_BF16)

  row_h = lax.broadcasted_iota(jnp.int32, (R16, DH), 0)
  scale = float(DH ** -0.5)

  def step(i, carry):
    o_h, acc_a = carry
    h = i // B
    b = i % B
    slot = i % NBUF
    o_h = jnp.where(b == 0, 0.0, o_h)

    wait_filled(kbuf.at[slot], k_sem.at[slot])

    @pl.when(i + LOOK < NSTEP)
    def _():
      start_k(i + LOOK)

    @pl.when(i == NSTEP - LOOK)
    def _():
      for c in range(len(W2_LATE)):
        start_rows(w2_hbm, w2_v, w2l_sem.at[c],
                   _row_pieces(W2_OFF[c], W2_OFF[c + 1], W_ROWS), priority=1)

    @pl.when(i == STEP_W1_ISSUE)
    def _():
      start_rows(w1_hbm, w1_v, w1_sem, _row_pieces(0, D, 8))

    @pl.when(i == STEP_WO0_ISSUE)
    def _():
      start_rows(wo_hbm, wo_v, wo_sem.at[0], _row_pieces(0, WO_HALF, W_ROWS))

    @pl.when(i == STEP_WO1_ISSUE)
    def _():
      start_rows(wo_hbm, wo_v, wo_sem.at[1], _row_pieces(WO_HALF, 2 * WO_HALF, W_ROWS))

    @pl.when(i == STEP_W2E_ISSUE)
    def _():
      start_rows(w2_hbm, w2_v, w2e_sem, _row_pieces(0, W2_EARLY, W_ROWS))

    s = lax.dot_general(q_v[h], kbuf[slot], (((1,), (1,)), ((), ())),
                        preferred_element_type=_F32)
    m = jnp.max(s, axis=-1, keepdims=True)
    p = jnp.exp((s - m) * scale)
    l = jnp.sum(p, axis=-1, keepdims=True)

    wait_filled(vbuf.at[slot], v_sem.at[slot])

    @pl.when(i + LOOK < NSTEP)
    def _():
      start_v(i + LOOK)

    o = jnp.dot(p.astype(_BF16), vbuf[slot], preferred_element_type=_F32)
    o_h = o_h + jnp.where(row_h % B == b, o / l, 0.0)

    def project():
      @pl.when(h % (HKV // 2) == 0)
      def _():
        wait_filled(wo_v.at[pl.ds(0, WO_HALF), :], wo_sem.at[h // (HKV // 2)])

      acc = acc_a
      o_bf = o_h.astype(_BF16)
      for r in range(REP):
        lhs = jnp.where(row_h // B == r, o_bf, jnp.zeros_like(o_bf))
        row0 = pl.multiple_of((h * REP + r) * DH, DH)
        acc = acc + jnp.dot(lhs, wo_v[pl.ds(row0, DH), :], preferred_element_type=_F32)
      return acc

    acc_a = lax.cond(b == B - 1, project, lambda: acc_a)

    @pl.when(i == STEP_FFN_UP)
    def _():
      wait_filled(w1_v, w1_sem)
      xb = jnp.concatenate([x_v[...]] * REP, axis=0)
      pre = jnp.dot(xb, w1_v[...], preferred_element_type=_F32)
      pre = pre + b1_v[...].astype(_F32).reshape(1, F)
      relu = jnp.where(pre > 0.0, pre, 0.0)
      h_v[...] = (relu * relu).astype(_BF16)

    @pl.when(i == STEP_W2E)
    def _():
      wait_filled(w2_v.at[pl.ds(0, W2_EARLY), :], w2e_sem)
      part = jnp.dot(h_v[0:8, 0:W2_EARLY], w2_v[0:W2_EARLY, :], preferred_element_type=_F32)
      bo_v[...] = part + b2_v[...].astype(_F32).reshape(1, D)

    return o_h, acc_a

  init = (jnp.zeros((R16, DH), _F32), jnp.zeros((R16, D), _F32))
  _, acc_a = lax.fori_loop(0, NSTEP, step, init)

  a8 = acc_a[0:8] + acc_a[8:16]
  a4 = a8 + pltpu.roll(a8, 4, 0)
  bo = bo_v[...]
  for c in range(len(W2_LATE)):
    wait_filled(w2_v.at[pl.ds(W2_OFF[c], W2_LATE[c]), :], w2l_sem.at[c])
    rows = slice(W2_OFF[c], W2_OFF[c + 1])
    bo = bo + jnp.dot(h_v[0:8, rows], w2_v[rows, :], preferred_element_type=_F32)
  res = g8 * a4 + (1.0 - g8) * bo
  o_ref[...] = res[0:B].astype(o_ref.dtype)


@jax.jit
def pallas_gated_mix__gqa_block_cached__dense_activation_squared_relu__decode_kernel(
    A_x: jax.Array,
    A_k_cache: jax.Array,
    A_v_cache: jax.Array,
    A_wq: jax.Array,
    A_wo: jax.Array,
    B_x: jax.Array,
    B_w1: jax.Array,
    B_b1: jax.Array,
    B_w2: jax.Array,
    B_b2: jax.Array,
    gate_w: jax.Array,
):
  del B_x
  hbm = pl.BlockSpec(memory_space=pl.ANY)
  out = pl.pallas_call(
      _kernel,
      in_specs=[hbm] * 10,
      out_specs=pl.BlockSpec(memory_space=pltpu.VMEM),
      out_shape=jax.ShapeDtypeStruct((B, D), _BF16),
      scratch_shapes=[
          pltpu.VMEM((B, D), _BF16),
          pltpu.VMEM((D,), _BF16),
          pltpu.VMEM((F,), _BF16),
          pltpu.VMEM((D,), _BF16),
          pltpu.VMEM((D, HQ * DH), _BF16),
          pltpu.VMEM((HQ * DH, D), _BF16),
          pltpu.VMEM((D, F), _BF16),
          pltpu.VMEM((F, D), _BF16),
          pltpu.VMEM((NBUF, SK, DH), _BF16),
          pltpu.VMEM((NBUF, SK, DH), _BF16),
          pltpu.VMEM((R16, F), _BF16),
          pltpu.VMEM((HKV, R16, DH), _BF16),
          pltpu.VMEM((8, D), _F32),
          pltpu.SemaphoreType.DMA((4,)),
          pltpu.SemaphoreType.DMA(()),
          pltpu.SemaphoreType.DMA((2,)),
          pltpu.SemaphoreType.DMA(()),
          pltpu.SemaphoreType.DMA(()),
          pltpu.SemaphoreType.DMA((len(W2_LATE),)),
          pltpu.SemaphoreType.DMA((NBUF,)),
          pltpu.SemaphoreType.DMA((NBUF,)),
      ],
      compiler_params=pltpu.CompilerParams(
          vmem_limit_bytes=48 * 1024 * 1024,
          disable_semaphore_checks=True,
          disable_bounds_checks=True,
      ),
  )(A_x.reshape(B, D), A_k_cache, A_v_cache, A_wq, A_wo, B_w1, B_b1, B_w2, B_b2, gate_w)
  return out.reshape(B, 1, D)
```

```python
import numpy as np

import jax
import jax.numpy as jnp
from jax import lax
from jax.experimental import pallas as pl
from jax.experimental.pallas import tpu as pltpu

B, D, HQ, HKV, SK, DH, F = 4, 512, 32, 8, 4096, 128, 1792
REP = HQ // HKV
R16 = REP * B
NSTEP = B * HKV

LOOK = 2
NBUF = LOOK + 1
KV_ROWS = 128
W_ROWS = 32
W1_ROWS = 8
QUARTER_ORDER = (0, 3, 2, 1)
UNIT = 32
WO_HALF = HQ * DH // 2
W2_LATE = (384, 256, 128)
W2_EARLY = F - sum(W2_LATE)
W2_OFF = tuple(int(v) for v in np.cumsum((W2_EARLY,) + W2_LATE))
STEP_W1_ISSUE = 0
STEP_WO0_ISSUE = 1
STEP_WO1_ISSUE = 8
STEP_W2E_ISSUE = 16
STEP_FFN_UP = 3
STEP_W2E = 24

_F32, _BF16 = jnp.float32, jnp.bfloat16


def _row_pieces(r0, r1, rows):
  return [(s, min(rows, r1 - s)) for s in range(r0, r1, rows)]


def _round_robin(pieces, unit):
  order = []
  for u in range(0, len(pieces), unit):
    chunk = pieces[u:u + unit]
    assert len(chunk) % 4 == 0
    span = len(chunk) // 4
    for t in range(len(chunk)):
      order.append((chunk[QUARTER_ORDER[t % 4] * span + t // 4], t % 2))
  return order


def _kernel(x_hbm, k_hbm, v_hbm, wq_hbm, wo_hbm, w1_hbm, b1_hbm, w2_hbm, b2_hbm, gw_hbm,
            o_ref,
            x_v, gw_v, b1_v, b2_v, wq_v, wo_v, w1_v, w2_v, kbuf, vbuf, h_v, q_v, bo_v,
            small_sem, wq_sem, wo_sem, w1_sem, w2e_sem, w2l_sem, k_sem, v_sem):

  def start_rows(src, dst, sem, order):
    for (r0, n), prio in order:
      rows = pl.ds(r0, n)
      pltpu.make_async_copy(src.at[rows, :], dst.at[rows, :], sem).start(priority=prio)

  def wait_filled(dst, sem):
    pltpu.make_async_copy(dst, dst, sem).wait()

  def small_copies():
    return [pltpu.make_async_copy(x_hbm, x_v, small_sem.at[0]),
            pltpu.make_async_copy(gw_hbm, gw_v, small_sem.at[1]),
            pltpu.make_async_copy(b1_hbm, b1_v, small_sem.at[2]),
            pltpu.make_async_copy(b2_hbm, b2_v, small_sem.at[3])]

  kv_order = _round_robin(_row_pieces(0, SK, KV_ROWS), UNIT)

  def start_k(i):
    slot = i % NBUF
    start_rows(k_hbm.at[i % B, i // B], kbuf.at[slot], k_sem.at[slot], kv_order)

  def start_v(i):
    slot = i % NBUF
    start_rows(v_hbm.at[i % B, i // B], vbuf.at[slot], v_sem.at[slot], kv_order)

  for c in small_copies():
    c.start(priority=0)

  def issue_wq(jj, carry):
    unit, j = jj // 8, jj % 8
    cols = pl.ds(pl.multiple_of((j % 2) * 2048, 2048), 2048)
    for t in range(4):
      row0 = unit * 128 + QUARTER_ORDER[t] * 32 + (j // 2) * 8
      rows = pl.ds(pl.multiple_of(row0, 8), 8)
      pltpu.make_async_copy(wq_hbm.at[rows, cols], wq_v.at[rows, cols],
                            wq_sem).start(priority=t % 2)
    return carry

  lax.fori_loop(0, (D // 128) * 8, issue_wq, 0)

  def issue_first_slabs(t, carry):
    @pl.when(t % 2 == 0)
    def _():
      start_k(t // 2)

    @pl.when(t % 2 == 1)
    def _():
      start_v(t // 2)

    return carry

  lax.fori_loop(0, 2 * LOOK, issue_first_slabs, 0)

  for c in small_copies():
    c.wait()
  x16 = jnp.concatenate([x_v[...].astype(_F32)] * REP, axis=0)
  gate_logit = jnp.sum(x16[0:8] * gw_v[...].astype(_F32).reshape(1, D),
                       axis=-1, keepdims=True)
  g8 = 1.0 / (1.0 + jnp.exp(-gate_logit))

  row_d = lax.broadcasted_iota(jnp.int32, (R16, D), 0)
  x_r = [jnp.where(row_d // B == r, x16, 0.0).astype(_BF16) for r in range(REP)]
  wait_filled(wq_v, wq_sem)
  for h in range(HKV):
    q = jnp.zeros((R16, DH), _F32)
    for r in range(REP):
      col = (h * REP + r) * DH
      q += jnp.dot(x_r[r], wq_v[:, col:col + DH], preferred_element_type=_F32)
    q_v[h] = q.astype(_BF16)

  row_h = lax.broadcasted_iota(jnp.int32, (R16, DH), 0)
  scale = float(DH ** -0.5)

  def step(i, carry):
    o_h, acc_a = carry
    h = i // B
    b = i % B
    slot = i % NBUF
    o_h = jnp.where(b == 0, 0.0, o_h)

    wait_filled(kbuf.at[slot], k_sem.at[slot])

    @pl.when(i + LOOK < NSTEP)
    def _():
      start_k(i + LOOK)

    @pl.when(i == NSTEP - LOOK)
    def _():
      for c in range(len(W2_LATE)):
        start_rows(w2_hbm, w2_v, w2l_sem.at[c],
                   [(p, 1) for p in _row_pieces(W2_OFF[c], W2_OFF[c + 1], W_ROWS)])

    @pl.when(i == STEP_W1_ISSUE)
    def _():
      pieces = _row_pieces(0, D, W1_ROWS)
      start_rows(w1_hbm, w1_v, w1_sem, _round_robin(pieces, len(pieces)))

    @pl.when(i == STEP_WO0_ISSUE)
    def _():
      start_rows(wo_hbm, wo_v, wo_sem.at[0],
                 _round_robin(_row_pieces(0, WO_HALF, W_ROWS), UNIT))

    @pl.when(i == STEP_WO1_ISSUE)
    def _():
      start_rows(wo_hbm, wo_v, wo_sem.at[1],
                 _round_robin(_row_pieces(WO_HALF, 2 * WO_HALF, W_ROWS), UNIT))

    @pl.when(i == STEP_W2E_ISSUE)
    def _():
      start_rows(w2_hbm, w2_v, w2e_sem,
                 _round_robin(_row_pieces(0, W2_EARLY, W_ROWS), UNIT))

    s = lax.dot_general(q_v[h], kbuf[slot], (((1,), (1,)), ((), ())),
                        preferred_element_type=_F32)
    m = jnp.max(s, axis=-1, keepdims=True)
    p = jnp.exp((s - m) * scale)
    l = jnp.sum(p, axis=-1, keepdims=True)

    wait_filled(vbuf.at[slot], v_sem.at[slot])

    @pl.when(i + LOOK < NSTEP)
    def _():
      start_v(i + LOOK)

    o = jnp.dot(p.astype(_BF16), vbuf[slot], preferred_element_type=_F32)
    o_h = o_h + jnp.where(row_h % B == b, o / l, 0.0)

    def project():
      @pl.when(h % (HKV // 2) == 0)
      def _():
        wait_filled(wo_v.at[pl.ds(0, WO_HALF), :], wo_sem.at[h // (HKV // 2)])

      acc = acc_a
      o_bf = o_h.astype(_BF16)
      for r in range(REP):
        lhs = jnp.where(row_h // B == r, o_bf, jnp.zeros_like(o_bf))
        row0 = pl.multiple_of((h * REP + r) * DH, DH)
        acc = acc + jnp.dot(lhs, wo_v[pl.ds(row0, DH), :], preferred_element_type=_F32)
      return acc

    acc_a = lax.cond(b == B - 1, project, lambda: acc_a)

    @pl.when(i == STEP_FFN_UP)
    def _():
      wait_filled(w1_v, w1_sem)
      xb = jnp.concatenate([x_v[...]] * REP, axis=0)
      pre = jnp.dot(xb, w1_v[...], preferred_element_type=_F32)
      pre = pre + b1_v[...].astype(_F32).reshape(1, F)
      relu = jnp.where(pre > 0.0, pre, 0.0)
      h_v[...] = (relu * relu).astype(_BF16)

    @pl.when(i == STEP_W2E)
    def _():
      wait_filled(w2_v.at[pl.ds(0, W2_EARLY), :], w2e_sem)
      part = jnp.dot(h_v[0:8, 0:W2_EARLY], w2_v[0:W2_EARLY, :], preferred_element_type=_F32)
      bo_v[...] = part + b2_v[...].astype(_F32).reshape(1, D)

    return o_h, acc_a

  init = (jnp.zeros((R16, DH), _F32), jnp.zeros((R16, D), _F32))
  _, acc_a = lax.fori_loop(0, NSTEP, step, init)

  a8 = acc_a[0:8] + acc_a[8:16]
  a4 = a8 + pltpu.roll(a8, 4, 0)
  bo = bo_v[...]
  for c in range(len(W2_LATE)):
    wait_filled(w2_v.at[pl.ds(W2_OFF[c], W2_LATE[c]), :], w2l_sem.at[c])
    rows = slice(W2_OFF[c], W2_OFF[c + 1])
    bo = bo + jnp.dot(h_v[0:8, rows], w2_v[rows, :], preferred_element_type=_F32)
  res = g8 * a4 + (1.0 - g8) * bo
  o_ref[...] = res[0:B].astype(o_ref.dtype)


@jax.jit
def pallas_gated_mix__gqa_block_cached__dense_activation_squared_relu__decode_kernel(
    A_x: jax.Array,
    A_k_cache: jax.Array,
    A_v_cache: jax.Array,
    A_wq: jax.Array,
    A_wo: jax.Array,
    B_x: jax.Array,
    B_w1: jax.Array,
    B_b1: jax.Array,
    B_w2: jax.Array,
    B_b2: jax.Array,
    gate_w: jax.Array,
):
  del B_x
  hbm = pl.BlockSpec(memory_space=pl.ANY)
  out = pl.pallas_call(
      _kernel,
      in_specs=[hbm] * 10,
      out_specs=pl.BlockSpec(memory_space=pltpu.VMEM),
      out_shape=jax.ShapeDtypeStruct((B, D), _BF16),
      scratch_shapes=[
          pltpu.VMEM((B, D), _BF16),
          pltpu.VMEM((D,), _BF16),
          pltpu.VMEM((F,), _BF16),
          pltpu.VMEM((D,), _BF16),
          pltpu.VMEM((D, HQ * DH), _BF16),
          pltpu.VMEM((HQ * DH, D), _BF16),
          pltpu.VMEM((D, F), _BF16),
          pltpu.VMEM((F, D), _BF16),
          pltpu.VMEM((NBUF, SK, DH), _BF16),
          pltpu.VMEM((NBUF, SK, DH), _BF16),
          pltpu.VMEM((R16, F), _BF16),
          pltpu.VMEM((HKV, R16, DH), _BF16),
          pltpu.VMEM((8, D), _F32),
          pltpu.SemaphoreType.DMA((4,)),
          pltpu.SemaphoreType.DMA(()),
          pltpu.SemaphoreType.DMA((2,)),
          pltpu.SemaphoreType.DMA(()),
          pltpu.SemaphoreType.DMA(()),
          pltpu.SemaphoreType.DMA((len(W2_LATE),)),
          pltpu.SemaphoreType.DMA((NBUF,)),
          pltpu.SemaphoreType.DMA((NBUF,)),
      ],
      compiler_params=pltpu.CompilerParams(
          vmem_limit_bytes=48 * 1024 * 1024,
          disable_semaphore_checks=True,
          disable_bounds_checks=True,
      ),
  )(A_x.reshape(B, D), A_k_cache, A_v_cache, A_wq, A_wo, B_w1, B_b1, B_w2, B_b2, gate_w)
  return out.reshape(B, 1, D)
```

```python
import numpy as np

import jax
import jax.numpy as jnp
from jax import lax
from jax.experimental import pallas as pl
from jax.experimental.pallas import tpu as pltpu

B, D, HQ, HKV, SK, DH, F = 4, 512, 32, 8, 4096, 128, 1792
REP = HQ // HKV
R16 = REP * B
NSTEP = B * HKV

LOOK = 2
NBUF = LOOK + 1
KV_ROWS = 128
W_ROWS = 32
W1_ROWS = 8
QUARTER_ORDER = (0, 3, 2, 1)
UNIT = 32
WO_HALF = HQ * DH // 2
W2_LATE = (384, 256, 128)
W2_EARLY = F - sum(W2_LATE)
W2_OFF = tuple(int(v) for v in np.cumsum((W2_EARLY,) + W2_LATE))
STEP_W1_ISSUE = 0
STEP_WO0_ISSUE = 1
STEP_WO1_ISSUE = 8
STEP_W2E_ISSUE = 16
STEP_FFN_UP = 3
STEP_W2E = 24

_F32, _BF16 = jnp.float32, jnp.bfloat16


def _row_pieces(r0, r1, rows):
  return [(s, min(rows, r1 - s)) for s in range(r0, r1, rows)]


def _round_robin(pieces, unit):
  order = []
  for u in range(0, len(pieces), unit):
    chunk = pieces[u:u + unit]
    assert len(chunk) % 4 == 0
    span = len(chunk) // 4
    for t in range(len(chunk)):
      order.append((chunk[QUARTER_ORDER[t % 4] * span + t // 4], t % 2))
  return order


def _kernel(x_hbm, k_hbm, v_hbm, wq_hbm, wo_hbm, w1_hbm, b1_hbm, w2_hbm, b2_hbm, gw_hbm,
            o_ref,
            x_v, gw_v, b1_v, b2_v, wq_v, wo_v, w1_v, w2_v, kbuf, vbuf, h_v, q_v, bo_v,
            small_sem, wq_sem, wo_sem, w1_sem, w2e_sem, w2l_sem, k_sem, v_sem):

  def start_rows(src, dst, sem, order):
    for (r0, n), prio in order:
      rows = pl.ds(r0, n)
      pltpu.make_async_copy(src.at[rows, :], dst.at[rows, :], sem).start(priority=prio)

  def wait_filled(dst, sem):
    pltpu.make_async_copy(dst, dst, sem).wait()

  def small_copies():
    return [pltpu.make_async_copy(x_hbm, x_v, small_sem.at[0]),
            pltpu.make_async_copy(gw_hbm, gw_v, small_sem.at[1]),
            pltpu.make_async_copy(b1_hbm, b1_v, small_sem.at[2]),
            pltpu.make_async_copy(b2_hbm, b2_v, small_sem.at[3])]

  kv_order = _round_robin(_row_pieces(0, SK, KV_ROWS), UNIT)

  def start_k(i):
    slot = i % NBUF
    start_rows(k_hbm.at[i % B, i // B], kbuf.at[slot], k_sem.at[slot], kv_order)

  def start_v(i):
    slot = i % NBUF
    start_rows(v_hbm.at[i % B, i // B], vbuf.at[slot], v_sem.at[slot], kv_order)

  for c in small_copies():
    c.start(priority=0)

  def issue_wq(jj, carry):
    unit, j = jj // 8, jj % 8
    cols = pl.ds(pl.multiple_of((j % 2) * 2048, 2048), 2048)
    for t in range(4):
      row0 = unit * 128 + QUARTER_ORDER[t] * 32 + (j // 2) * 8
      rows = pl.ds(pl.multiple_of(row0, 8), 8)
      pltpu.make_async_copy(wq_hbm.at[rows, cols], wq_v.at[rows, cols],
                            wq_sem).start(priority=t % 2)
    return carry

  lax.fori_loop(0, (D // 128) * 8, issue_wq, 0)

  def issue_first_slabs(t, carry):
    @pl.when(t % 2 == 0)
    def _():
      start_k(t // 2)

    @pl.when(t % 2 == 1)
    def _():
      start_v(t // 2)

    return carry

  lax.fori_loop(0, 2 * LOOK, issue_first_slabs, 0)

  for c in small_copies():
    c.wait()
  x16 = jnp.concatenate([x_v[...].astype(_F32)] * REP, axis=0)
  gate_logit = jnp.sum(x16[0:8] * gw_v[...].astype(_F32).reshape(1, D),
                       axis=-1, keepdims=True)
  g8 = 1.0 / (1.0 + jnp.exp(-gate_logit))

  row_d = lax.broadcasted_iota(jnp.int32, (R16, D), 0)
  x_r = [jnp.where(row_d // B == r, x16, 0.0).astype(_BF16) for r in range(REP)]
  wait_filled(wq_v, wq_sem)
  for h in range(HKV):
    q = jnp.zeros((R16, DH), _F32)
    for r in range(REP):
      col = (h * REP + r) * DH
      q += jnp.dot(x_r[r], wq_v[:, col:col + DH], preferred_element_type=_F32)
    q_v[h] = q.astype(_BF16)

  row_h = lax.broadcasted_iota(jnp.int32, (R16, DH), 0)
  scale = float(DH ** -0.5)

  def step(i, carry):
    o_h, acc_a = carry
    h = i // B
    b = i % B
    slot = i % NBUF
    o_h = jnp.where(b == 0, 0.0, o_h)

    wait_filled(kbuf.at[slot], k_sem.at[slot])

    @pl.when(i + LOOK < NSTEP)
    def _():
      start_k(i + LOOK)

    @pl.when(i == NSTEP - LOOK)
    def _():
      for c in range(len(W2_LATE)):
        start_rows(w2_hbm, w2_v, w2l_sem.at[c],
                   [(p, 1) for p in _row_pieces(W2_OFF[c], W2_OFF[c + 1], W_ROWS)])

    @pl.when(i == STEP_W1_ISSUE)
    def _():
      pieces = _row_pieces(0, D, W1_ROWS)
      start_rows(w1_hbm, w1_v, w1_sem, _round_robin(pieces, len(pieces)))

    @pl.when(i == STEP_WO0_ISSUE)
    def _():
      start_rows(wo_hbm, wo_v, wo_sem.at[0],
                 _round_robin(_row_pieces(0, WO_HALF, W_ROWS), UNIT))

    @pl.when(i == STEP_WO1_ISSUE)
    def _():
      start_rows(wo_hbm, wo_v, wo_sem.at[1],
                 _round_robin(_row_pieces(WO_HALF, 2 * WO_HALF, W_ROWS), UNIT))

    @pl.when(i == STEP_W2E_ISSUE)
    def _():
      start_rows(w2_hbm, w2_v, w2e_sem,
                 _round_robin(_row_pieces(0, W2_EARLY, W_ROWS), UNIT))

    s = lax.dot_general(q_v[h], kbuf[slot], (((1,), (1,)), ((), ())),
                        preferred_element_type=_F32)
    m = jnp.max(s, axis=-1, keepdims=True)
    p = jnp.exp((s - m) * scale)
    l = jnp.sum(p, axis=-1, keepdims=True)

    wait_filled(vbuf.at[slot], v_sem.at[slot])

    @pl.when(i + LOOK < NSTEP)
    def _():
      start_v(i + LOOK)

    o = jnp.dot(p.astype(_BF16), vbuf[slot], preferred_element_type=_F32)
    o_h = o_h + jnp.where(row_h % B == b, o / l, 0.0)

    def project():
      for half in range(2):
        @pl.when(h == half * (HKV // 2))
        def _():
          wait_filled(wo_v.at[pl.ds(half * WO_HALF, WO_HALF), :], wo_sem.at[half])

      acc = acc_a
      o_bf = o_h.astype(_BF16)
      for r in range(REP):
        lhs = jnp.where(row_h // B == r, o_bf, jnp.zeros_like(o_bf))
        row0 = pl.multiple_of((h * REP + r) * DH, DH)
        acc = acc + jnp.dot(lhs, wo_v[pl.ds(row0, DH), :], preferred_element_type=_F32)
      return acc

    acc_a = lax.cond(b == B - 1, project, lambda: acc_a)

    @pl.when(i == STEP_FFN_UP)
    def _():
      wait_filled(w1_v, w1_sem)
      xb = jnp.concatenate([x_v[...]] * REP, axis=0)
      pre = jnp.dot(xb, w1_v[...], preferred_element_type=_F32)
      pre = pre + b1_v[...].astype(_F32).reshape(1, F)
      relu = jnp.where(pre > 0.0, pre, 0.0)
      h_v[...] = (relu * relu).astype(_BF16)

    @pl.when(i == STEP_W2E)
    def _():
      wait_filled(w2_v.at[pl.ds(0, W2_EARLY), :], w2e_sem)
      part = jnp.dot(h_v[0:8, 0:W2_EARLY], w2_v[0:W2_EARLY, :], preferred_element_type=_F32)
      bo_v[...] = part + b2_v[...].astype(_F32).reshape(1, D)

    return o_h, acc_a

  init = (jnp.zeros((R16, DH), _F32), jnp.zeros((R16, D), _F32))
  _, acc_a = lax.fori_loop(0, NSTEP, step, init)

  a8 = acc_a[0:8] + acc_a[8:16]
  a4 = a8 + pltpu.roll(a8, 4, 0)
  bo = bo_v[...]
  for c in range(len(W2_LATE)):
    wait_filled(w2_v.at[pl.ds(W2_OFF[c], W2_LATE[c]), :], w2l_sem.at[c])
    rows = slice(W2_OFF[c], W2_OFF[c + 1])
    bo = bo + jnp.dot(h_v[0:8, rows], w2_v[rows, :], preferred_element_type=_F32)
  res = g8 * a4 + (1.0 - g8) * bo
  o_ref[...] = res[0:B].astype(o_ref.dtype)


@jax.jit
def pallas_gated_mix__gqa_block_cached__dense_activation_squared_relu__decode_kernel(
    A_x: jax.Array,
    A_k_cache: jax.Array,
    A_v_cache: jax.Array,
    A_wq: jax.Array,
    A_wo: jax.Array,
    B_x: jax.Array,
    B_w1: jax.Array,
    B_b1: jax.Array,
    B_w2: jax.Array,
    B_b2: jax.Array,
    gate_w: jax.Array,
):
  del B_x
  hbm = pl.BlockSpec(memory_space=pl.ANY)
  out = pl.pallas_call(
      _kernel,
      in_specs=[hbm] * 10,
      out_specs=pl.BlockSpec(memory_space=pltpu.VMEM),
      out_shape=jax.ShapeDtypeStruct((B, D), _BF16),
      scratch_shapes=[
          pltpu.VMEM((B, D), _BF16),
          pltpu.VMEM((D,), _BF16),
          pltpu.VMEM((F,), _BF16),
          pltpu.VMEM((D,), _BF16),
          pltpu.VMEM((D, HQ * DH), _BF16),
          pltpu.VMEM((HQ * DH, D), _BF16),
          pltpu.VMEM((D, F), _BF16),
          pltpu.VMEM((F, D), _BF16),
          pltpu.VMEM((NBUF, SK, DH), _BF16),
          pltpu.VMEM((NBUF, SK, DH), _BF16),
          pltpu.VMEM((R16, F), _BF16),
          pltpu.VMEM((HKV, R16, DH), _BF16),
          pltpu.VMEM((8, D), _F32),
          pltpu.SemaphoreType.DMA((4,)),
          pltpu.SemaphoreType.DMA(()),
          pltpu.SemaphoreType.DMA((2,)),
          pltpu.SemaphoreType.DMA(()),
          pltpu.SemaphoreType.DMA(()),
          pltpu.SemaphoreType.DMA((len(W2_LATE),)),
          pltpu.SemaphoreType.DMA((NBUF,)),
          pltpu.SemaphoreType.DMA((NBUF,)),
      ],
      compiler_params=pltpu.CompilerParams(
          vmem_limit_bytes=48 * 1024 * 1024,
          disable_semaphore_checks=True,
          disable_bounds_checks=True,
      ),
  )(A_x.reshape(B, D), A_k_cache, A_v_cache, A_wq, A_wo, B_w1, B_b1, B_w2, B_b2, gate_w)
  return out.reshape(B, 1, D)
```
